```python
import os as _os
_os.environ.setdefault('JAX_PLATFORMS', 'cpu')
import jax
import jax.numpy as jnp

def _softmax(x, axis=-1):
    return jax.nn.softmax(x, axis=axis)

def _gelu(x):
    return jax.nn.gelu(x, approximate=True)

def _silu(x):
    return jax.nn.silu(x)

def _sigmoid(x):
    return jax.nn.sigmoid(x)

def _layernorm(x, axis=-1, eps=1e-05):
    m = jnp.mean(x, axis=axis, keepdims=True)
    v = jnp.var(x, axis=axis, keepdims=True)
    return (x - m) / jnp.sqrt(v + eps)

def _scatter_add(tgt, idx, src, axis=0):
    return tgt.at[idx].add(src)

def _segment_sum(src, seg, n):
    return jax.ops.segment_sum(src, seg, n)

class _Rng:

    def __init__(self, key):
        self._k = key

    def _next(self):
        self._k, sub = jax.random.split(self._k)
        return sub

    def normal(self, shape):
        return jax.random.normal(self._next(), shape, dtype=jnp.bfloat16)

    def randint(self, lo, hi, shape):
        return jax.random.randint(self._next(), shape, lo, hi, dtype=jnp.int32)

    def uniform(self, shape, lo=0.0, hi=1.0):
        return jax.random.uniform(self._next(), shape, jnp.bfloat16, lo, hi)

    def permutation(self, n):
        return jax.random.permutation(self._next(), n)
kernel_name = 'parallel_sum__memory_aug_recurrent_mem_tr__dense_activation_silu__prompt'

def setup_inputs():
    _rng = _Rng(jax.random.key(int.from_bytes(__import__("os").urandom(4), "little")))
    _w = lambda a: (lambda t: t.astype(jnp.bfloat16) if jnp.issubdtype(t.dtype, jnp.floating) else t)(jnp.asarray(a))

    def _A_setup():
        B, S, Dm = (1, 2048, 448)
        H, Dh = (16, 256)
        M, seg = (8, 32)
        seg = min(seg, S)
        S = S // seg * seg
        return {'x': _w((lambda *s: _rng.normal(s) * 0.05)(B, S, Dm)), 'mem0': _w((lambda *s: _rng.normal(s) * 0.2)(B, M, Dm)), 'Wq': _w((lambda *s: _rng.normal(s) * 0.8)(Dm, H, Dh) * Dm ** (-0.5)), 'Wk': _w((lambda *s: _rng.normal(s) * 0.8)(Dm, H, Dh) * Dm ** (-0.5)), 'Wv': _w((lambda *s: _rng.normal(s) * 0.2)(Dm, H, Dh) * Dm ** (-0.5)), 'Wo': _w((lambda *s: _rng.normal(s) * 0.2)(H, Dh, Dm) * (H * Dh) ** (-0.5)), 'seg_len': seg}
    _A_in = _A_setup()

    def _B_setup():
        B, S, D, F = (1, 2048, 448, 1792)
        return {'x': _w((lambda *s: _rng.normal(s) * 0.05)(B, S, D)), 'w1': _w((lambda *s: _rng.normal(s) * 0.05)(D, F) * D ** (-0.5)), 'w2': _w((lambda *s: _rng.normal(s) * 0.05)(F, D) * F ** (-0.5))}
    _B_in = _B_setup()
    return {'A_x': _A_in['x'], 'A_mem0': _A_in['mem0'], 'A_Wq': _A_in['Wq'], 'A_Wk': _A_in['Wk'], 'A_Wv': _A_in['Wv'], 'A_Wo': _A_in['Wo'], 'A_seg_len': _A_in['seg_len'], 'B_x': _B_in['x'], 'B_w1': _B_in['w1'], 'B_w2': _B_in['w2']}

def reference(A_x, A_mem0, A_Wq, A_Wk, A_Wv, A_Wo, A_seg_len, B_x, B_w1, B_w2):

    def _A_ref(x, mem0, Wq, Wk, Wv, Wo, seg_len):
        B, S, Dm = x.shape
        H, Dh = (Wq.shape[1], Wq.shape[2])
        M = mem0.shape[1]
        scale = Dh ** (-0.5)
        n_seg = S // seg_len
        L = M + seg_len
        idx = jnp.arange(L)
        mask = (idx[:, None] < M) | (idx[:, None] >= idx[None, :])
        mem = mem0
        outs = []
        for s in range(n_seg):
            xs = x[:, s * seg_len:(s + 1) * seg_len, :].copy()
            h = jnp.concatenate([mem, xs], axis=1)
            q = jnp.einsum('btd,dhe->bhte', h, Wq)
            k = jnp.einsum('btd,dhe->bhte', h, Wk)
            v = jnp.einsum('btd,dhe->bhte', h, Wv)
            scores = jnp.einsum('bhqe,bhke->bhqk', q, k) * scale
            scores = jnp.where(mask[None, None], scores, -1000000000.0)
            p = _softmax(scores, axis=-1)
            o = jnp.einsum('bhqk,bhke->bhqe', p, v)
            o = jnp.einsum('bhte,hed->btd', o, Wo)
            mem = o[:, :M, :].copy()
            outs.append(o[:, M:, :])
        return jnp.concatenate(outs, axis=1)

    def _B_ref(x, w1, w2):
        h = jnp.einsum('bsd,df->bsf', x, w1)
        h = _silu(h)
        out = jnp.einsum('bsf,fd->bsd', h, w2)
        return out
    x = A_x
    xn = _layernorm(x, axis=-1)
    return x + _A_ref(xn, A_mem0, A_Wq, A_Wk, A_Wv, A_Wo, A_seg_len) + _B_ref(xn, B_w1, B_w2)
```

```python
import functools
import contextlib
import jax
import jax.numpy as jnp
import numpy as np
from jax.experimental import pallas as pl
from jax.experimental.pallas import tpu as pltpu

D = 448
NH = 16
DH = 256
FF = 1792
SEQ = 2048
SEG = 32
MM = 8
DP = 512
NTP = 56
NG = SEQ // 128
BF = jnp.bfloat16
F32 = jnp.float32
NT_DIMS = (((1,), (1,)), ((), ()))
DCH = [(0, 128), (128, 128), (256, 128), (384, 64)]

def _K(t): return [f"K{t}{c}" for c in range(4 if t < 3 else 2)]
def _V(t): return [f"V{t}{c}" for c in range(4 if t < 3 else 2)]
_KALL = _K(0) + _K(1) + ["X"] + _K(2) + _K(3)
_SALL = ["S0", "S1", "S2", "S3", "S4"]
PROG = {
    "v1": _KALL + _V(0) + _SALL + _V(1) + ["M"] + _V(2) + ["P0", "P1"] + _V(3) + ["P2", "F", "P3", "F"],
    "v3": _KALL + _V(0) + _SALL + ["M"] + _V(1) + _V(2) + _V(3) + ["P0", "P1", "P2", "F", "P3", "F"],
    "i1": _KALL + ["V00", "S0", "V01", "S1", "V02", "S2", "V03", "S3", "V10", "S4", "M", "V11", "V12", "V13"] + _V(2) + _V(3) + ["P0", "P1", "P2", "F", "P3", "F"],
    "i2": _KALL + ["V00", "S0", "V01", "S1", "V02", "S2", "V03", "S3", "V10", "S4", "M", "V11", "V12", "V13"] + _V(2) + ["V30", "P0", "V31", "P1", "F", "P2", "P3", "F"],
    "i3": _KALL + ["V00", "S0", "V01", "S1", "V02", "S2", "V03", "S3", "V10", "S4", "M", "V11", "V12", "V13"] + _V(2) + ["V30", "P0", "V31", "P1", "P2", "F", "P3", "F"],
    "i4": _KALL + ["V00", "S0", "V01", "S1", "V02", "S2", "V03", "S3", "V10", "S4", "M", "V11", "V12", "V13", "V20", "V21", "V22", "P0", "V23", "V30", "P1", "V31", "P2", "F", "P3", "F"],
    "i5": _KALL + ["V00", "S0", "V01", "S1", "V02", "S2", "V03", "S3", "V10", "S4", "M", "V11", "V12", "V13", "V20", "V21", "P0", "V22", "V23", "P1", "V30", "V31", "P2", "F", "P3", "F"],
}


def _grp8_allreduce(x, op, lane):
    for s in (1, 2, 4):
        up = pltpu.roll(x, 128 - s, axis=1)
        dn = pltpu.roll(x, s, axis=1)
        x = op(x, jnp.where((lane & s) == 0, up, dn))
    return x


def make_kernel(chunk_tiles=4, mask_val=-1e9, scopes=True, order="v1", outpos=0, lnpos=1, fmode="a", dbg=""):
    NS = jax.named_scope if scopes else (lambda n: contextlib.nullcontext())

    def kernel(xt_hbm, mem0_ref, wq_hbm, wk_hbm, wv_hbm, wo_hbm, w1_hbm, w2t_hbm, o_hbm,
               xt_v, wq0, wq1, wk0, wk1, wv0, wv1, wo_v, w1_v, w2t_v, wqd, wkd,
               wcat, xn_ref, ka, va, kb, vb, att_ref, y_ref, h1_ref, sems):
        scale = DH ** -0.5
        semc = [0]

        def mk(src, dst):
            c = pltpu.make_async_copy(src, dst, sems.at[semc[0]])
            semc[0] += 1
            return c

        def chunk_copies(src, d0, d1, c):
            r0, nr = DCH[c]
            return [mk(src.at[r0 * NH:(r0 + nr) * NH, hf * 128:(hf + 1) * 128], dst.at[r0 * NH:(r0 + nr) * NH, :])
                    for hf, dst in enumerate((d0, d1))]

        cv = [chunk_copies(wv_hbm, wv0, wv1, c) for c in range(4)]
        co = [mk(wo_hbm.at[p * 2 * D:(p + 1) * 2 * D, :], wo_v.at[p * 2 * D:(p + 1) * 2 * D, :]) for p in range(8)]
        cq = [chunk_copies(wq_hbm, wq0, wq1, c) for c in range(4)]
        ck = [chunk_copies(wk_hbm, wk0, wk1, c) for c in range(4)]
        cx0 = mk(xt_hbm.at[:, 0:256], xt_v.at[:, 0:256])
        cxr = mk(xt_hbm.at[:, 256:SEQ], xt_v.at[:, 256:SEQ])
        c1 = mk(w1_hbm, w1_v)
        c2 = mk(w2t_hbm, w2t_v)
        so = semc[0]
        dma_order = (cv[0] + co[0:2] + cv[1] + co[2:4] + cv[2] + co[4:6] + cv[3] + co[6:8]
                     + cq[0] + ck[0] + cq[1] + ck[1] + cq[2] + ck[2] + cq[3] + ck[3] + [cx0, c1, c2, cxr])
        for c in dma_order:
            c.start()

        def heads(b0, b1, hp, r0, nr):
            los, his = [], []
            for b in (b0, b1):
                v = b.bitcast(jnp.uint32)[pl.ds(r0 * 8 + hp, nr, stride=8), :]
                los.append(pltpu.bitcast(v << 16, F32).astype(BF))
                his.append(pltpu.bitcast(v & jnp.uint32(0xFFFF0000), F32).astype(BF))
            return jnp.concatenate(los, axis=1), jnp.concatenate(his, axis=1)

        lo64 = {}
        def lomask(nr):
            if nr not in lo64:
                lo64[nr] = jax.lax.broadcasted_iota(jnp.int32, (nr, 128), 1) < 64
            return lo64[nr]

        def vunit(c, p):
            r0, nr = DCH[c]
            a = 2 * p
            wva, wvb = heads(wv0, wv1, p, r0, nr)
            fa = jax.lax.dot_general(wva, wo_v[a * D:(a + 1) * D, :], NT_DIMS, preferred_element_type=F32)
            fb = jax.lax.dot_general(wvb, wo_v[(a + 1) * D:(a + 2) * D, :], NT_DIMS, preferred_element_type=F32)
            for h, f in ((a, fa), (a + 1, fb)):
                for t in range(3):
                    col = (NTP + t * NH + h) * 128
                    wcat[r0:r0 + nr, col:col + 128] = f[:, t * 128:(t + 1) * 128].astype(BF)
            col = (NTP + 48 + p) * 128
            wcat[r0:r0 + nr, col:col + 128] = jnp.concatenate([fa[:, 384:448], fb[:, 384:448]], axis=1).astype(BF)

        with NS("foldv"):
            att_ref[...] = jnp.zeros((128, DP), F32)
            y_ref[...] = jnp.zeros((D, 128), F32)
            vplan = [
                (cv[0] + co[0:2], [(0, 0), (0, 1)]),
                (cv[1], [(1, 0), (1, 1)]),
                (co[2:4], [(0, 2), (1, 2), (0, 3), (1, 3)]),
                (cv[2], [(2, 0), (2, 1), (2, 2), (2, 3)]),
                (co[4:6], [(0, 4), (1, 4), (2, 4), (0, 5), (1, 5), (2, 5)]),
                (cv[3] + co[6:8], [(0, 6), (1, 6), (2, 6), (0, 7), (1, 7), (2, 7)] + [(3, p) for p in range(8)]),
            ]
            for waits, units in vplan:
                for d_ in waits:
                    d_.wait()
                for (cc, p) in units:
                    vunit(cc, p)

        def split(b0, b1, dst, c):
            r0, nr = DCH[c]
            for hp in range(8):
                qa, qb = heads(b0, b1, hp, r0, nr)
                dst[(2 * hp) * D + r0:(2 * hp) * D + r0 + nr, :] = qa
                dst[(2 * hp + 1) * D + r0:(2 * hp + 1) * D + r0 + nr, :] = qb

        def kunit(cg, cf):
            r0, nr = DCH[cg]
            f0, nf = DCH[cf]
            for p in range(8):
                a = 2 * p
                fa = jax.lax.dot_general(wkd[a * D + r0:a * D + r0 + nr, :], wqd[a * D + f0:a * D + f0 + nf, :], NT_DIMS, preferred_element_type=F32) * scale
                fb = jax.lax.dot_general(wkd[(a + 1) * D + r0:(a + 1) * D + r0 + nr, :], wqd[(a + 1) * D + f0:(a + 1) * D + f0 + nf, :], NT_DIMS, preferred_element_type=F32) * scale
                if cf < 3:
                    wcat[r0:r0 + nr, (cf * NH + a) * 128:(cf * NH + a + 1) * 128] = fa.astype(BF)
                    wcat[r0:r0 + nr, (cf * NH + a + 1) * 128:(cf * NH + a + 2) * 128] = fb.astype(BF)
                else:
                    wcat[r0:r0 + nr, (48 + p) * 128:(49 + p) * 128] = jnp.concatenate([fa, fb], axis=1).astype(BF)

        with NS("foldk"):
            kplan = [
                (cq[0] + ck[0] + cq[1], [("q", 0), ("k", 0), ("q", 1), (0, 0), (0, 1)]),
                (ck[1], [("k", 1), (1, 0), (1, 1)]),
                (cq[2], [("q", 2), (0, 2), (1, 2)]),
                (ck[2], [("k", 2), (2, 0), (2, 1), (2, 2)]),
                (cq[3] + ck[3], [("q", 3), ("k", 3), (0, 3), (1, 3), (2, 3), (3, 0), (3, 1), (3, 2), (3, 3)]),
            ]
            for waits, units in kplan:
                for d_ in waits:
                    d_.wait()
                for u_ in units:
                    if u_[0] == "q":
                        split(wq0, wq1, wqd, u_[1])
                    elif u_[0] == "k":
                        split(wk0, wk1, wkd, u_[1])
                    else:
                        kunit(*u_)

        def ln_group(c0):
            xc = xt_v[:, pl.ds(c0, 128)].astype(F32)
            mu = jnp.mean(xc, axis=0, keepdims=True)
            x0 = xc - mu
            var = jnp.mean(x0 * x0, axis=0, keepdims=True)
            xn = x0 * jax.lax.rsqrt(var + 1e-5)
            for t in range(3):
                xn_ref[pl.ds(c0, 128), t * 128:(t + 1) * 128] = xn[t * 128:(t + 1) * 128, :].T
            xl = xn[384:448, :]
            xn_ref[pl.ds(c0, 128), 384:512] = jnp.concatenate([xl, xl], axis=0).T

        with NS("ln0"):
            cx0.wait()
            ln_group(0)
            c1.wait()
            c2.wait()

        lane = jax.lax.broadcasted_iota(jnp.int32, (8, 128), 1)
        sub = jax.lax.broadcasted_iota(jnp.int32, (8, 128), 0)
        diag_mask = (lane & 7) <= sub
        lane40 = jax.lax.broadcasted_iota(jnp.int32, (40, 128), 1)

        def proj(hb, rowmap, part, t, ci):
            R = hb.shape[0]
            ntile = NH if t < 3 else NH // 2
            if t == 3:
                lo = lomask(R)
            for c0 in [ci * chunk_tiles]:
                tile0 = part * NTP + t * NH + c0
                y = jnp.dot(hb, wcat[:, tile0 * 128:(tile0 + chunk_tiles) * 128], preferred_element_type=F32)
                if t < 3:
                    for q in range(chunk_tiles // 2):
                        a = c0 + 2 * q
                        ya = y[:, (2 * q) * 128:(2 * q + 1) * 128]
                        yb = y[:, (2 * q + 1) * 128:(2 * q + 2) * 128]
                        for r, (ks, vs, jh) in enumerate(rowmap):
                            blk = jnp.concatenate([ya[8 * r:8 * r + 8], yb[8 * r:8 * r + 8]], axis=0)
                            dst = ks if part == 0 else vs
                            dst[jh * 128 + a * 8:jh * 128 + a * 8 + 16, t * 128:(t + 1) * 128] = blk.astype(BF)
                else:
                    for q in range(chunk_tiles):
                        a = 2 * (c0 + q)
                        yt = y[:, q * 128:(q + 1) * 128]
                        ya = jnp.where(lo, yt, 0.0)
                        yb = jnp.where(lo, 0.0, yt)
                        for r, (ks, vs, jh) in enumerate(rowmap):
                            blk = jnp.concatenate([ya[8 * r:8 * r + 8], yb[8 * r:8 * r + 8]], axis=0)
                            dst = ks if part == 0 else vs
                            dst[jh * 128 + a * 8:jh * 128 + a * 8 + 16, 384:512] = blk.astype(BF)

        def scores(hq, ks):
            return jax.lax.dot_general(hq, ks[...], NT_DIMS, preferred_element_type=F32)

        def softmax(s):
            if "nosm" in dbg:
                return (s * 0.01).astype(BF)
            tl, ms = [], []
            for ih in range(5):
                jhs = range(5) if ih == 0 else range(ih + 1)
                row = []
                for jh in jhs:
                    tt = s[8 * ih:8 * ih + 8, 128 * jh:128 * (jh + 1)]
                    if ih > 0 and jh == ih:
                        tt = jnp.where(diag_mask, tt, mask_val)
                    row.append(tt)
                tl.append(row)
                ms.append(functools.reduce(jnp.maximum, row))
            m = _grp8_allreduce(jnp.concatenate(ms, axis=0), jnp.maximum, lane40)
            es, ls = [], []
            for ih in range(5):
                mi = m[8 * ih:8 * ih + 8]
                row = [jnp.exp(tt - mi) for tt in tl[ih]]
                es.append(row)
                ls.append(functools.reduce(jnp.add, row))
            l = _grp8_allreduce(jnp.concatenate(ls, axis=0), jnp.add, lane40)
            r = 1.0 / l
            rows = []
            for ih in range(5):
                ri = r[8 * ih:8 * ih + 8]
                row = [e * ri for e in es[ih]]
                row += [jnp.zeros((8, 128), F32)] * (5 - len(row))
                rows.append(jnp.concatenate(row, axis=1))
            rows.append(jnp.zeros((8, 640), F32))
            return jnp.concatenate(rows, axis=0).astype(BF)

        def pv(p, vs, t):
            o = jnp.dot(p, vs[:, t * 128:(t + 1) * 128], preferred_element_type=F32)[0:40]
            if t == 3:
                o = o + pltpu.roll(o, 64, axis=1)
            return o

        F1 = [(0, 4), (4, 3), (7, 4), (11, 3)]

        def ffn1(g, piece):
            n0, nn = F1[piece]
            xb = xn_ref[pl.ds(pl.multiple_of(g * 128, 128), 128), :].astype(BF)[:, 0:D]
            h = jnp.dot(xb, w1_v[:, n0 * 128:(n0 + nn) * 128], preferred_element_type=F32)
            h1_ref[:, n0 * 128:(n0 + nn) * 128] = (h * jax.nn.sigmoid(h)).astype(BF)

        def ffn2(piece):
            rows = D // 4
            r0 = piece * rows
            y = jax.lax.dot_general(w2t_v[r0:r0 + rows, :], h1_ref[...], NT_DIMS, preferred_element_type=F32)
            y_ref[r0:r0 + rows, :] = y

        def out_copy(g):
            c0 = pl.multiple_of(g * 128, 128)
            return pltpu.make_async_copy(xt_v.at[:, pl.ds(c0, 128)], o_hbm.at[:, pl.ds(c0, 128)], sems.at[so + g % 2])

        def out_stage(gs, gx):
            c0 = pl.multiple_of(gx * 128, 128)
            c1 = pl.multiple_of(gs * 128, 128)
            for t in range(4):
                at = att_ref[:, t * 128:(t + 1) * 128].T
                n = 128 if t < 3 else 64
                res = at[0:n] + y_ref[t * 128:t * 128 + n, :] + xt_v[t * 128:t * 128 + n, pl.ds(c0, 128)].astype(F32)
                xt_v[t * 128:t * 128 + n, pl.ds(c1, 128)] = res.astype(BF)

        def step(hproj, hq, rowmap, ks, vs, fillers, side, prog):
            f = list(fillers)
            st = {}
            sp = {}
            os_ = {}
            cur = [None]
            def enter(name):
                if cur[0] is not None:
                    cur[0].__exit__(None, None, None)
                    cur[0] = None
                if name is not None and "sc" in dbg:
                    cur[0] = jax.named_scope(name)
                    cur[0].__enter__()
            R_ = hproj.shape[0]
            enter(f"K{R_}")
            seenV = False
            seenP = False
            for tok in prog:
                k = tok[0]
                if k == "V" and not seenV:
                    seenV = True
                    enter(f"V{R_}")
                if k == "P" and not seenP:
                    seenP = True
                    enter(f"P{R_}")
                if k == "K":
                    proj(hproj, rowmap, 0, int(tok[1]), int(tok[2]))
                elif k == "V":
                    proj(hproj, rowmap, 1, int(tok[1]), int(tok[2]))
                elif k == "S" and "noS" in dbg:
                    j = int(tok[1])
                    sp[j] = hq[:, 0:128].astype(F32)
                elif k == "S":
                    j = int(tok[1])
                    sp[j] = jax.lax.dot_general(hq, ks[j * 128:(j + 1) * 128, :], NT_DIMS, preferred_element_type=F32)
                elif k == "M":
                    st["p"] = softmax(jnp.concatenate([sp[j] for j in range(5)], axis=1))
                elif k == "P" and "noP" in dbg:
                    t = int(tok[1])
                    os_[t] = st["p"][0:40, t * 128:(t + 1) * 128].astype(F32)
                elif k == "P":
                    t = int(tok[1])
                    os_[t] = pv(st["p"], vs, t)
                elif k == "F":
                    if f:
                        f.pop(0)()
                elif k == "X":
                    if side is not None:
                        side()
                else:
                    raise ValueError(tok)
            while f:
                f.pop(0)()
            enter(None)
            return jnp.concatenate([os_[t] for t in range(4)], axis=1)

        def body(g, mem):
            gp = (g + NG - 1) % NG
            gn = jnp.minimum(g + 1, NG - 1)
            fills = [
                [lambda: ffn1(g, 0), lambda: ffn1(g, 1)],
                [lambda: ffn1(g, 2), lambda: ffn1(g, 3)],
                [lambda: ffn2(0), lambda: ffn2(1)],
                [lambda: ffn2(2), lambda: ffn2(3)],
            ]
            if "noffn" in dbg:
                fills = [[], [], [], []]
            sides = [None] * 4
            sides[0] = lambda: out_stage(jnp.where(g > 0, g - 1, NG), jnp.maximum(g - 1, 0))
            ln_side = lambda: ln_group(pl.multiple_of(gn * 128, 128))
            sides[lnpos] = ln_side
            if "noln" in dbg:
                sides[lnpos] = None
            if False:
                pass
            for u in range(2):
                t0 = pl.multiple_of(g * 128 + 64 * u, 64)
                ha = jnp.concatenate([mem, xn_ref[pl.ds(t0, 40), :]], axis=0).astype(BF)
                oa = step(ha[:, 0:D], ha,
                          [(ka, va, 0), (ka, va, 1), (ka, va, 2), (ka, va, 3), (ka, va, 4), (kb, vb, 1)],
                          ka, va, fills[2 * u], sides[2 * u], PROG[order])
                memb = oa[0:8]
                if "nodep" in dbg:
                    memb = xn_ref[pl.ds(t0, 8), :] * 0.5
                    att_ref[0:8, :] = oa[0:8]
                att_ref[64 * u:64 * u + 32, :] = oa[8:40]
                hb = jnp.concatenate([memb, xn_ref[pl.ds(t0 + 40, 24), :]], axis=0).astype(BF)
                hq = jnp.concatenate([memb, xn_ref[pl.ds(t0 + 32, 32), :], jnp.zeros((8, DP), F32)], axis=0).astype(BF)
                ob = step(hb[:, 0:D], hq, [(kb, vb, 0), (kb, vb, 2), (kb, vb, 3), (kb, vb, 4)],
                          kb, vb, fills[2 * u + 1], sides[2 * u + 1], PROG[order])
                mem = ob[0:8]
                if "nodep" in dbg:
                    mem = xn_ref[pl.ds(t0 + 8, 8), :] * 0.5
                    att_ref[8:16, :] = ob[0:8]
                att_ref[64 * u + 32:64 * u + 64, :] = ob[8:40]
            @pl.when(g == 0)
            def _():
                cxr.wait()

            @pl.when(g > 0)
            def _():
                out_copy(g - 1).start()

            @pl.when(g > 1)
            def _():
                out_copy(g - 2).wait()
            return mem

        with NS("main"):
            m0 = mem0_ref[...].astype(F32)
            ml = m0[:, 384:448]
            mem_init = jnp.concatenate([m0[:, 0:384], ml, ml], axis=1)
            jax.lax.fori_loop(0, NG, body, mem_init)
        with NS("tail"):
            out_stage(NG - 1, NG - 1)
            out_copy(NG - 1).start()
            out_copy(NG - 2).wait()
            out_copy(NG - 1).wait()

    return kernel


def build(**kw):
    kern = make_kernel(**kw)

    def f(A_x, A_mem0, A_Wq, A_Wk, A_Wv, A_Wo, B_w1, B_w2):
        xt = jnp.swapaxes(A_x, 1, 2).reshape(D, SEQ)
        mem0 = A_mem0.reshape(MM, D)
        wq = A_Wq.reshape(D * NH, DH)
        wk = A_Wk.reshape(D * NH, DH)
        wv = A_Wv.reshape(D * NH, DH)
        wo = jnp.swapaxes(A_Wo, 1, 2).reshape(NH * D, DH)
        w2t = jnp.swapaxes(B_w2, 0, 1)
        anyspec = pl.BlockSpec(memory_space=pl.ANY)
        out = pl.pallas_call(
            kern,
            out_shape=jax.ShapeDtypeStruct((D, SEQ), BF),
            in_specs=[anyspec, pl.BlockSpec(memory_space=pltpu.VMEM), anyspec, anyspec, anyspec, anyspec, anyspec, anyspec],
            out_specs=anyspec,
            scratch_shapes=[
                pltpu.VMEM((D, SEQ + 128), BF),
                pltpu.VMEM((D * NH, 128), BF), pltpu.VMEM((D * NH, 128), BF),
                pltpu.VMEM((D * NH, 128), BF), pltpu.VMEM((D * NH, 128), BF),
                pltpu.VMEM((D * NH, 128), BF), pltpu.VMEM((D * NH, 128), BF),
                pltpu.VMEM((NH * D, DH), BF),
                pltpu.VMEM((D, FF), BF), pltpu.VMEM((D, FF), BF),
                pltpu.VMEM((NH * D, DH), BF), pltpu.VMEM((NH * D, DH), BF),
                pltpu.VMEM((D, 2 * NTP * 128), BF),
                pltpu.VMEM((SEQ, DP), F32),
                pltpu.VMEM((640, DP), BF), pltpu.VMEM((640, DP), BF),
                pltpu.VMEM((640, DP), BF), pltpu.VMEM((640, DP), BF),
                pltpu.VMEM((128, DP), F32),
                pltpu.VMEM((D, 128), F32),
                pltpu.VMEM((128, FF), BF),
                pltpu.SemaphoreType.DMA((48,)),
            ],
            compiler_params=pltpu.CompilerParams(vmem_limit_bytes=100 * 1024 * 1024),
        )(xt, mem0, wq, wk, wv, wo, B_w1, w2t)
        return jnp.swapaxes(out.reshape(1, D, SEQ), 1, 2)
    return f


_impl = build(**{"order":"v3","scopes":False,"lnpos":3})


@functools.partial(jax.jit, static_argnames=("A_seg_len",))
def pallas_parallel_sum__memory_aug_recurrent_mem_tr__dense_activation_silu__prompt_kernel(
    A_x: jax.Array,
    A_mem0: jax.Array,
    A_Wq: jax.Array,
    A_Wk: jax.Array,
    A_Wv: jax.Array,
    A_Wo: jax.Array,
    A_seg_len: int,
    B_x: jax.Array,
    B_w1: jax.Array,
    B_w2: jax.Array,
):
    assert A_seg_len == SEG and A_x.shape == (1, SEQ, D) and A_mem0.shape == (1, MM, D)
    assert A_Wq.shape == (D, NH, DH) and B_w1.shape == (D, FF)
    return _impl(A_x, A_mem0, A_Wq, A_Wk, A_Wv, A_Wo, B_w1, B_w2)
```

```python
import functools

import jax
import jax.numpy as jnp
from jax.experimental import pallas as pl
from jax.experimental.pallas import tpu as pltpu

D = 448
NH = 16
DH = 256
FF = 1792
SEQ = 2048
SEG = 32
MM = 8
DP = 512
NTP = 56
NG = SEQ // 128
BF = jnp.bfloat16
F32 = jnp.float32
NT_DIMS = (((1,), (1,)), ((), ()))
DCH = [(0, 128), (128, 128), (256, 128), (384, 64)]
SCALE = DH ** -0.5
MASK_VAL = -1e9 / SCALE
EXP2_SCALE = SCALE * 1.4426950408889634

F1_PIECES = [(0, 3), (3, 2), (5, 2), (7, 3), (10, 2), (12, 2)]
F2_PIECES = [(0, 80), (80, 64), (144, 80), (224, 80), (304, 64), (368, 80)]

PROG_A = ["K02", "K00", "K10", "K21", "K03", "K01", "K11", "K12", "K20", "V31", "K13", "K22", "V00", "K31",
          "K30", "K23", "V30", "S0", "V02", "S1", "V12", "V03", "S2", "S3", "V01", "V10", "V11", "S4", "M",
          "V23", "V13", "X", "V22", "V20", "V21", "P3", "F", "P0", "P2", "P1", "F", "F"]
PROG_B = ["K10", "K00", "K01", "K02", "K03", "K11", "K31", "K12", "K30", "K21", "K13", "K20", "K23", "K22",
          "V00", "V01", "V03", "V10", "V02", "F", "S3", "S1", "S0", "S2", "V11", "S4", "V12", "V30", "M",
          "V13", "V20", "X", "V21", "V22", "V23", "V31", "P0", "P1", "F", "P3", "P2", "F"]


def _grp8_allreduce(x, op, lane):
    for s in (1, 2, 4):
        up = pltpu.roll(x, 128 - s, axis=1)
        dn = pltpu.roll(x, s, axis=1)
        x = op(x, jnp.where((lane & s) == 0, up, dn))
    return x


def _nt(a, b):
    return jax.lax.dot_general(a, b, NT_DIMS, preferred_element_type=F32)


def _kernel(xt_hbm, mem0_ref, wq_hbm, wk_hbm, wv_hbm, wo_hbm, w1_hbm, w2t_hbm, o_hbm,
            xt_v, wq0, wq1, wk0, wk1, wv0, wv1, wo_v, w1_v, w2t_v, wqd,
            wcat, xn_ref, ka, va, kb, vb, att_ref, y_ref, h1_ref, sems):
    semc = [0]

    def mk(src, dst):
        c = pltpu.make_async_copy(src, dst, sems.at[semc[0]])
        semc[0] += 1
        return c

    def chunk_copies(src, d0, d1, c):
        r0, nr = DCH[c]
        return [mk(src.at[r0 * NH:(r0 + nr) * NH, hf * 128:(hf + 1) * 128], dst.at[r0 * NH:(r0 + nr) * NH, :])
                for hf, dst in enumerate((d0, d1))]

    cv = [chunk_copies(wv_hbm, wv0, wv1, c) for c in range(4)]
    co = [mk(wo_hbm.at[p * 2 * D:(p + 1) * 2 * D, :], wo_v.at[p * 2 * D:(p + 1) * 2 * D, :]) for p in range(8)]
    cq = [chunk_copies(wq_hbm, wq0, wq1, c) for c in range(4)]
    ck = [chunk_copies(wk_hbm, wk0, wk1, c) for c in range(4)]
    cx0 = mk(xt_hbm.at[:, 0:256], xt_v.at[:, 0:256])
    cxr = mk(xt_hbm.at[:, 256:SEQ], xt_v.at[:, 256:SEQ])
    c1 = mk(w1_hbm, w1_v)
    c2 = mk(w2t_hbm, w2t_v)
    so = semc[0]
    for c in (cv[0] + co[0:2] + cv[1] + co[2:4] + cv[2] + co[4:6] + cv[3] + co[6:8]
              + cq[0] + cq[3] + ck[0] + cq[1] + ck[1] + cq[2] + ck[2] + ck[3] + [cx0, c1, c2, cxr]):
        c.start()

    def wait(*copies):
        for c in copies:
            c.wait()

    def heads(b0, b1, hp, r0, nr):
        los, his = [], []
        for b in (b0, b1):
            v = b.bitcast(jnp.uint32)[pl.ds(r0 * 8 + hp, nr, stride=8), :]
            los.append(jax.lax.bitcast_convert_type(v.astype(jnp.uint16), BF))
            his.append(jax.lax.bitcast_convert_type((v >> 16).astype(jnp.uint16), BF))
        return jnp.concatenate(los, axis=1), jnp.concatenate(his, axis=1)

    def tlast(la, lb, ra, rb):
        return jnp.concatenate([_nt(la, ra), _nt(lb, rb)], axis=0).T.astype(BF)

    def vunit(c, p):
        r0, nr = DCH[c]
        a = 2 * p
        wva, wvb = heads(wv0, wv1, p, r0, nr)
        if nr == 128:
            fa = _nt(wva, wo_v[a * D:a * D + 384, :])
            fb = _nt(wvb, wo_v[(a + 1) * D:(a + 1) * D + 384, :])
            last = tlast(wo_v[a * D + 384:(a + 1) * D, :], wo_v[(a + 1) * D + 384:(a + 2) * D, :], wva, wvb)
        else:
            fa = _nt(wva, wo_v[a * D:(a + 1) * D, :])
            fb = _nt(wvb, wo_v[(a + 1) * D:(a + 2) * D, :])
            last = jnp.concatenate([fa[:, 384:448], fb[:, 384:448]], axis=1).astype(BF)
        for h, f in ((a, fa), (a + 1, fb)):
            for t in range(3):
                col = (NTP + t * NH + h) * 128
                wcat[r0:r0 + nr, col:col + 128] = f[:, t * 128:(t + 1) * 128].astype(BF)
        col = (NTP + 48 + p) * 128
        wcat[r0:r0 + nr, col:col + 128] = last

    def vunits(chunks, pairs):
        for p in pairs:
            for c in chunks:
                vunit(c, p)

    def split_q(c):
        r0, nr = DCH[c]
        for hp in range(8):
            qa, qb = heads(wq0, wq1, hp, r0, nr)
            wqd[(2 * hp) * D + r0:(2 * hp) * D + r0 + nr, :] = qa
            wqd[(2 * hp + 1) * D + r0:(2 * hp + 1) * D + r0 + nr, :] = qb

    def kunit(r0, nr, f0, nf):
        for p in range(8):
            a = 2 * p
            wka, wkb = heads(wk0, wk1, p, r0, nr)
            has_last = f0 + nf > 384
            transposed_last = has_last and nr % 128 == 0
            nfull = (min(f0 + nf, 384) - f0) // 128 if f0 < 384 else 0
            nfm = nfull * 128 if transposed_last else nf
            if nfm > 0:
                fa = _nt(wka, wqd[a * D + f0:a * D + f0 + nfm, :])
                fb = _nt(wkb, wqd[(a + 1) * D + f0:(a + 1) * D + f0 + nfm, :])
            for j in range(nfull):
                cf = f0 // 128 + j
                wcat[r0:r0 + nr, (cf * NH + a) * 128:(cf * NH + a + 1) * 128] = fa[:, j * 128:(j + 1) * 128].astype(BF)
                wcat[r0:r0 + nr, (cf * NH + a + 1) * 128:(cf * NH + a + 2) * 128] = fb[:, j * 128:(j + 1) * 128].astype(BF)
            if transposed_last:
                for i in range(nr // 128):
                    wcat[r0 + i * 128:r0 + (i + 1) * 128, (48 + p) * 128:(49 + p) * 128] = tlast(
                        wqd[a * D + 384:(a + 1) * D, :], wqd[(a + 1) * D + 384:(a + 2) * D, :],
                        wka[i * 128:(i + 1) * 128], wkb[i * 128:(i + 1) * 128])
            elif has_last:
                o = 384 - f0
                wcat[r0:r0 + nr, (48 + p) * 128:(49 + p) * 128] = jnp.concatenate(
                    [fa[:, o:o + 64], fb[:, o:o + 64]], axis=1).astype(BF)

    def colsum(v):
        p = [v[64 * i:64 * (i + 1)] for i in range(7)]
        q = ((p[0] + p[1]) + (p[2] + p[3])) + ((p[4] + p[5]) + p[6])
        r = (q[0:8] + q[8:16]) + (q[16:24] + q[24:32])
        r2 = (q[32:40] + q[40:48]) + (q[48:56] + q[56:64])
        return jnp.sum(r + r2, axis=0, keepdims=True)

    def layernorm(c0):
        xc = xt_v[:, pl.ds(c0, 128)].astype(F32)
        mu = colsum(xc) * (1.0 / D)
        x0 = xc - mu
        var = colsum(x0 * x0) * (1.0 / D)
        xn = x0 * jax.lax.rsqrt(var + 1e-5)
        for t in range(3):
            xn_ref[pl.ds(c0, 128), t * 128:(t + 1) * 128] = xn[t * 128:(t + 1) * 128, :].T
        xl = xn[384:448, :]
        xn_ref[pl.ds(c0, 128), 384:512] = jnp.concatenate([xl, xl], axis=0).T

    att_ref[...] = jnp.zeros((128, DP), BF)
    y_ref[...] = jnp.zeros((D, 128), F32)

    wait(*cv[0], co[0], co[1]); vunits([0], [0, 1])
    wait(*cv[1]); vunits([1], [0, 1])
    wait(co[2], co[3]); vunits([0, 1], [2, 3])
    wait(*cv[2]); vunits([2], [0, 1, 2, 3])
    wait(co[4], co[5]); vunits([0, 1, 2], [4, 5])
    wait(*cv[3], co[6], co[7]); vunits([0, 1, 2], [6, 7])
    vunits([3], [0, 1, 2, 3, 4, 5, 6, 7])

    wait(*cq[0], *cq[3], *ck[0]); split_q(0); kunit(0, 128, 0, 128); split_q(3)
    wait(*cq[1]); split_q(1); kunit(0, 128, 384, 64); kunit(0, 128, 128, 128)
    wait(*ck[1]); kunit(128, 128, 0, 256)
    wait(*cq[2]); split_q(2); kunit(128, 128, 384, 64); kunit(0, 256, 256, 128)
    wait(*ck[2]); kunit(256, 128, 0, 448)
    wait(*ck[3], cx0); layernorm(0); kunit(384, 64, 0, 448)
    wait(c1, c2)

    lane = jax.lax.broadcasted_iota(jnp.int32, (8, 128), 1)
    sub = jax.lax.broadcasted_iota(jnp.int32, (8, 128), 0)
    diag_mask = (lane & 7) <= sub
    lane40 = jax.lax.broadcasted_iota(jnp.int32, (40, 128), 1)
    lo_masks = {}

    def lo_mask(nr):
        if nr not in lo_masks:
            lo_masks[nr] = jax.lax.broadcasted_iota(jnp.int32, (nr, 128), 1) < 64
        return lo_masks[nr]

    def project(hb, rowmap, part, t, ci):
        tile0 = part * NTP + t * NH + ci * 4
        y = jnp.dot(hb, wcat[:, tile0 * 128:(tile0 + 4) * 128], preferred_element_type=F32)
        if t < 3:
            for q in range(2):
                a = ci * 4 + 2 * q
                ya = y[:, (2 * q) * 128:(2 * q + 1) * 128]
                yb = y[:, (2 * q + 1) * 128:(2 * q + 2) * 128]
                for r, (ks, vs, jh) in enumerate(rowmap):
                    blk = jnp.concatenate([ya[8 * r:8 * r + 8], yb[8 * r:8 * r + 8]], axis=0)
                    dst = ks if part == 0 else vs
                    dst[jh * 128 + a * 8:jh * 128 + a * 8 + 16, t * 128:(t + 1) * 128] = blk.astype(BF)
        else:
            lo = lo_mask(hb.shape[0])
            for q in range(4):
                a = 2 * (ci * 4 + q)
                yt = y[:, q * 128:(q + 1) * 128]
                ya = jnp.where(lo, yt, 0.0)
                yb = jnp.where(lo, 0.0, yt)
                for r, (ks, vs, jh) in enumerate(rowmap):
                    blk = jnp.concatenate([ya[8 * r:8 * r + 8], yb[8 * r:8 * r + 8]], axis=0)
                    dst = ks if part == 0 else vs
                    dst[jh * 128 + a * 8:jh * 128 + a * 8 + 16, 384:512] = blk.astype(BF)

    def softmax(s):
        tiles, ms = [], []
        for ih in range(5):
            row = []
            for jh in (range(5) if ih == 0 else range(ih + 1)):
                tt = s[8 * ih:8 * ih + 8, 128 * jh:128 * (jh + 1)]
                if ih > 0 and jh == ih:
                    tt = jnp.where(diag_mask, tt, MASK_VAL)
                row.append(tt)
            tiles.append(row)
            ms.append(functools.reduce(jnp.maximum, row))
        m = _grp8_allreduce(jnp.concatenate(ms, axis=0), jnp.maximum, lane40)
        es, ls = [], []
        for ih in range(5):
            mi = m[8 * ih:8 * ih + 8]
            row = [jnp.exp2((tt - mi) * EXP2_SCALE) for tt in tiles[ih]]
            es.append(row)
            ls.append(functools.reduce(jnp.add, row))
        r = 1.0 / _grp8_allreduce(jnp.concatenate(ls, axis=0), jnp.add, lane40)
        rows = []
        for ih in range(5):
            ri = r[8 * ih:8 * ih + 8]
            row = [e * ri for e in es[ih]]
            row += [jnp.zeros((8, 128), F32)] * (5 - len(row))
            rows.append(jnp.concatenate(row, axis=1))
        rows.append(jnp.zeros((8, 640), F32))
        return jnp.concatenate(rows, axis=0).astype(BF)

    def pv(p, vs, t):
        o = jnp.dot(p, vs[:, t * 128:(t + 1) * 128], preferred_element_type=F32)[0:40]
        if t == 3:
            o = o + pltpu.roll(o, 64, axis=1)
        return o

    def ffn1(g, n0, nn):
        xb = xn_ref[pl.ds(pl.multiple_of(g * 128, 128), 128), :].astype(BF)[:, 0:D]
        h = jnp.dot(xb, w1_v[:, n0 * 128:(n0 + nn) * 128], preferred_element_type=F32)
        h1_ref[:, n0 * 128:(n0 + nn) * 128] = (h * jax.nn.sigmoid(h)).astype(BF)

    def ffn2(r0, rows):
        y_ref[r0:r0 + rows, :] = _nt(w2t_v[r0:r0 + rows, :], h1_ref[...])

    def out_copy(g):
        c0 = pl.multiple_of(g * 128, 128)
        return pltpu.make_async_copy(xt_v.at[:, pl.ds(c0, 128)], o_hbm.at[:, pl.ds(c0, 128)], sems.at[so + g % 2])

    def out_stage(gs, gx):
        c0 = pl.multiple_of(gx * 128, 128)
        c1 = pl.multiple_of(gs * 128, 128)
        for t in range(4):
            n = 128 if t < 3 else 64
            at = att_ref[:, t * 128:(t + 1) * 128].astype(F32).T[0:n]
            res = at + y_ref[t * 128:t * 128 + n, :] + xt_v[t * 128:t * 128 + n, pl.ds(c0, 128)].astype(F32)
            xt_v[t * 128:t * 128 + n, pl.ds(c1, 128)] = res.astype(BF)

    def step(hproj, hq, rowmap, ks, vs, fillers, side, prog):
        fillers = list(fillers)
        sc, outs, prob = {}, {}, None
        for tok in prog:
            kind = tok[0]
            if kind == "K":
                project(hproj, rowmap, 0, int(tok[1]), int(tok[2]))
            elif kind == "V":
                project(hproj, rowmap, 1, int(tok[1]), int(tok[2]))
            elif kind == "S":
                j = int(tok[1])
                sc[j] = _nt(hq, ks[j * 128:(j + 1) * 128, :])
            elif kind == "M":
                prob = softmax(jnp.concatenate([sc[j] for j in range(5)], axis=1))
            elif kind == "P":
                outs[int(tok[1])] = pv(prob, vs, int(tok[1]))
            elif kind == "F":
                fillers.pop(0)()
            elif side is not None:
                side()
        return jnp.concatenate([outs[t] for t in range(4)], axis=1)

    def group(g, mem):
        gn = jnp.minimum(g + 1, NG - 1)
        f1 = [functools.partial(ffn1, g, n0, nn) for (n0, nn) in F1_PIECES]
        f2 = [functools.partial(ffn2, r0, nr) for (r0, nr) in F2_PIECES]
        fills = [f1[:3], f1[3:], f2[:3], f2[3:]]
        sides = [lambda: out_stage(jnp.where(g > 0, g - 1, NG), jnp.maximum(g - 1, 0)), None,
                 lambda: layernorm(pl.multiple_of(gn * 128, 128)), None]
        for u in range(2):
            t0 = pl.multiple_of(g * 128 + 64 * u, 64)
            ha = jnp.concatenate([mem, xn_ref[pl.ds(t0, 40), :]], axis=0).astype(BF)
            oa = step(ha[:, 0:D], ha,
                      [(ka, va, 0), (ka, va, 1), (ka, va, 2), (ka, va, 3), (ka, va, 4), (kb, vb, 1)],
                      ka, va, fills[2 * u], sides[2 * u], PROG_A)
            memb = oa[0:8]
            att_ref[64 * u:64 * u + 32, :] = oa[8:40].astype(BF)
            hb = jnp.concatenate([memb, xn_ref[pl.ds(t0 + 40, 24), :]], axis=0).astype(BF)
            hq = jnp.concatenate([memb, xn_ref[pl.ds(t0 + 32, 32), :], jnp.zeros((8, DP), F32)], axis=0).astype(BF)
            ob = step(hb[:, 0:D], hq, [(kb, vb, 0), (kb, vb, 2), (kb, vb, 3), (kb, vb, 4)],
                      kb, vb, fills[2 * u + 1], sides[2 * u + 1], PROG_B)
            mem = ob[0:8]
            att_ref[64 * u + 32:64 * u + 64, :] = ob[8:40].astype(BF)

        @pl.when(g == 0)
        def _():
            cxr.wait()

        @pl.when(g > 0)
        def _():
            out_copy(g - 1).start()

        @pl.when(g > 1)
        def _():
            out_copy(g - 2).wait()

        return mem

    m0 = mem0_ref[...].astype(F32)
    ml = m0[:, 384:448]
    jax.lax.fori_loop(0, NG, group, jnp.concatenate([m0[:, 0:384], ml, ml], axis=1))

    out_stage(NG - 1, NG - 1)
    out_copy(NG - 1).start()
    out_copy(NG - 2).wait()
    out_copy(NG - 1).wait()


def _forward(A_x, A_mem0, A_Wq, A_Wk, A_Wv, A_Wo, B_w1, B_w2):
    xt = jnp.swapaxes(A_x, 1, 2).reshape(D, SEQ)
    mem0 = A_mem0.reshape(MM, D)
    wq = A_Wq.reshape(D * NH, DH)
    wk = A_Wk.reshape(D * NH, DH)
    wv = A_Wv.reshape(D * NH, DH)
    wo = jnp.swapaxes(A_Wo, 1, 2).reshape(NH * D, DH)
    w2t = jnp.swapaxes(B_w2, 0, 1)
    hbm = pl.BlockSpec(memory_space=pl.ANY)
    half = pltpu.VMEM((D * NH + 64, 128), BF)
    out = pl.pallas_call(
        _kernel,
        out_shape=jax.ShapeDtypeStruct((D, SEQ), BF),
        in_specs=[hbm, pl.BlockSpec(memory_space=pltpu.VMEM), hbm, hbm, hbm, hbm, hbm, hbm],
        out_specs=hbm,
        scratch_shapes=[
            pltpu.VMEM((D, SEQ + 128), BF),
            half, half, half, half, half, half,
            pltpu.VMEM((NH * D, DH), BF),
            pltpu.VMEM((D, FF), BF), pltpu.VMEM((D, FF), BF),
            pltpu.VMEM((NH * D, DH), BF),
            pltpu.VMEM((D, 2 * NTP * 128), BF),
            pltpu.VMEM((SEQ, DP), F32),
            pltpu.VMEM((640, DP), BF), pltpu.VMEM((640, DP), BF),
            pltpu.VMEM((640, DP), BF), pltpu.VMEM((640, DP), BF),
            pltpu.VMEM((128, DP), BF),
            pltpu.VMEM((D, 128), F32),
            pltpu.VMEM((128, FF), BF),
            pltpu.SemaphoreType.DMA((38,)),
        ],
        compiler_params=pltpu.CompilerParams(vmem_limit_bytes=100 * 1024 * 1024),
    )(xt, mem0, wq, wk, wv, wo, B_w1, w2t)
    return jnp.swapaxes(out.reshape(1, D, SEQ), 1, 2)


@functools.partial(jax.jit, static_argnames=("A_seg_len",))
def pallas_parallel_sum__memory_aug_recurrent_mem_tr__dense_activation_silu__prompt_kernel(
    A_x: jax.Array,
    A_mem0: jax.Array,
    A_Wq: jax.Array,
    A_Wk: jax.Array,
    A_Wv: jax.Array,
    A_Wo: jax.Array,
    A_seg_len: int,
    B_x: jax.Array,
    B_w1: jax.Array,
    B_w2: jax.Array,
):
    assert A_seg_len == SEG and A_x.shape == (1, SEQ, D) and A_mem0.shape == (1, MM, D)
    assert A_Wq.shape == (D, NH, DH) and B_w1.shape == (D, FF)
    return _forward(A_x, A_mem0, A_Wq, A_Wk, A_Wv, A_Wo, B_w1, B_w2)
```

```python
import functools

import jax
import jax.numpy as jnp
from jax.experimental import pallas as pl
from jax.experimental.pallas import tpu as pltpu

D = 448
NH = 16
DH = 256
FF = 1792
SEQ = 2048
SEG = 32
MM = 8
DP = 512
NTP = 56
NG = SEQ // 128
BF = jnp.bfloat16
F32 = jnp.float32
NT_DIMS = (((1,), (1,)), ((), ()))
DCH = [(0, 128), (128, 128), (256, 128), (384, 64)]
SCALE = DH ** -0.5
MASK_VAL = -1e9 / SCALE
EXP2_SCALE = SCALE * 1.4426950408889634

F1_PIECES = [(0, 1), (1, 3), (4, 3), (7, 1), (8, 3), (11, 3)]
F2_PIECES = [(0, 80), (80, 64), (144, 80), (224, 80), (304, 64), (368, 80)]

PROG_A = ["K10", "K02", "K00", "K21", "K03", "K01", "K11", "K12", "K20", "V31", "V00", "K31", "K13", "K22",
          "K30", "K23", "V30", "S0", "V02", "S1", "V12", "V03", "S3", "V01", "V10", "V11", "S2", "S4", "M",
          "V23", "V13", "X", "V22", "V20", "V21", "P3", "F", "P0", "P2", "P1", "F", "F"]
PROG_B = ["K10", "K00", "K01", "K02", "K03", "K11", "K31", "K12", "K30", "K21", "K13", "K20", "K23", "K22",
          "V00", "V01", "V03", "V10", "V02", "F", "S3", "S1", "S0", "S2", "V11", "S4", "V12", "V30", "M", "V20",
          "V22", "V13", "X", "V21", "V23", "V31", "P0", "P1", "F", "P3", "P2", "F"]


def _grp8_allreduce(x, op, lane):
    for s in (1, 2, 4):
        up = pltpu.roll(x, 128 - s, axis=1)
        dn = pltpu.roll(x, s, axis=1)
        x = op(x, jnp.where((lane & s) == 0, up, dn))
    return x


def _nt(a, b):
    return jax.lax.dot_general(a, b, NT_DIMS, preferred_element_type=F32)


def _kernel(xt_hbm, mem0_ref, wq_hbm, wk_hbm, wv_hbm, wo_hbm, w1_hbm, w2t_hbm, o_hbm,
            xt_v, wq0, wq1, wk0, wk1, wv0, wv1, wo_v, w1_v, w2t_v, wqd,
            wcat, xn_ref, ka, va, kb, vb, att_ref, y_ref, h1_ref, sems):
    semc = [0]

    def mk(src, dst):
        c = pltpu.make_async_copy(src, dst, sems.at[semc[0]])
        semc[0] += 1
        return c

    def chunk_copies(src, d0, d1, c):
        r0, nr = DCH[c]
        return [mk(src.at[r0 * NH:(r0 + nr) * NH, hf * 128:(hf + 1) * 128], dst.at[r0 * NH:(r0 + nr) * NH, :])
                for hf, dst in enumerate((d0, d1))]

    cv = [chunk_copies(wv_hbm, wv0, wv1, c) for c in range(4)]
    co = [mk(wo_hbm.at[p * 2 * D:(p + 1) * 2 * D, :], wo_v.at[p * 2 * D:(p + 1) * 2 * D, :]) for p in range(8)]
    cq = [chunk_copies(wq_hbm, wq0, wq1, c) for c in range(4)]
    ck = [chunk_copies(wk_hbm, wk0, wk1, c) for c in range(4)]
    cx0 = mk(xt_hbm.at[:, 0:256], xt_v.at[:, 0:256])
    cxr = mk(xt_hbm.at[:, 256:SEQ], xt_v.at[:, 256:SEQ])
    c1 = mk(w1_hbm, w1_v)
    c2 = mk(w2t_hbm, w2t_v)
    so = semc[0]
    for c in (cv[0] + co[0:2] + cv[1] + co[2:4] + cv[2] + co[4:6] + cv[3] + co[6:8]
              + cq[0] + cq[3] + ck[0] + cq[1] + ck[1] + cq[2] + ck[2] + ck[3] + [cx0, c1, c2, cxr]):
        c.start()

    def wait(*copies):
        for c in copies:
            c.wait()

    def heads(b0, b1, hp, r0, nr):
        los, his = [], []
        for b in (b0, b1):
            v = b.bitcast(jnp.uint32)[pl.ds(r0 * 8 + hp, nr, stride=8), :]
            los.append(jax.lax.bitcast_convert_type(v.astype(jnp.uint16), BF))
            his.append(jax.lax.bitcast_convert_type((v >> 16).astype(jnp.uint16), BF))
        return jnp.concatenate(los, axis=1), jnp.concatenate(his, axis=1)

    def tlast(la, lb, ra, rb):
        return jnp.concatenate([_nt(la, ra), _nt(lb, rb)], axis=0).T.astype(BF)

    def vunit(c, p):
        r0, nr = DCH[c]
        a = 2 * p
        wva, wvb = heads(wv0, wv1, p, r0, nr)
        if nr == 128:
            fa = _nt(wva, wo_v[a * D:a * D + 384, :])
            fb = _nt(wvb, wo_v[(a + 1) * D:(a + 1) * D + 384, :])
            last = tlast(wo_v[a * D + 384:(a + 1) * D, :], wo_v[(a + 1) * D + 384:(a + 2) * D, :], wva, wvb)
        else:
            fa = _nt(wva, wo_v[a * D:(a + 1) * D, :])
            fb = _nt(wvb, wo_v[(a + 1) * D:(a + 2) * D, :])
            last = jnp.concatenate([fa[:, 384:448], fb[:, 384:448]], axis=1).astype(BF)
        for h, f in ((a, fa), (a + 1, fb)):
            for t in range(3):
                col = (NTP + t * NH + h) * 128
                wcat[r0:r0 + nr, col:col + 128] = f[:, t * 128:(t + 1) * 128].astype(BF)
        col = (NTP + 48 + p) * 128
        wcat[r0:r0 + nr, col:col + 128] = last

    def vunits(chunks, pairs):
        for p in pairs:
            for c in chunks:
                vunit(c, p)

    def split_q(c):
        r0, nr = DCH[c]
        for hp in range(8):
            qa, qb = heads(wq0, wq1, hp, r0, nr)
            wqd[(2 * hp) * D + r0:(2 * hp) * D + r0 + nr, :] = qa
            wqd[(2 * hp + 1) * D + r0:(2 * hp + 1) * D + r0 + nr, :] = qb

    def kunit(r0, nr, f0, nf):
        for p in range(8):
            a = 2 * p
            wka, wkb = heads(wk0, wk1, p, r0, nr)
            has_last = f0 + nf > 384
            transposed_last = has_last and nr % 128 == 0
            nfull = (min(f0 + nf, 384) - f0) // 128 if f0 < 384 else 0
            nfm = nfull * 128 if transposed_last else nf
            if nfm > 0:
                fa = _nt(wka, wqd[a * D + f0:a * D + f0 + nfm, :])
                fb = _nt(wkb, wqd[(a + 1) * D + f0:(a + 1) * D + f0 + nfm, :])
            for j in range(nfull):
                cf = f0 // 128 + j
                wcat[r0:r0 + nr, (cf * NH + a) * 128:(cf * NH + a + 1) * 128] = fa[:, j * 128:(j + 1) * 128].astype(BF)
                wcat[r0:r0 + nr, (cf * NH + a + 1) * 128:(cf * NH + a + 2) * 128] = fb[:, j * 128:(j + 1) * 128].astype(BF)
            if transposed_last:
                for i in range(nr // 128):
                    wcat[r0 + i * 128:r0 + (i + 1) * 128, (48 + p) * 128:(49 + p) * 128] = tlast(
                        wqd[a * D + 384:(a + 1) * D, :], wqd[(a + 1) * D + 384:(a + 2) * D, :],
                        wka[i * 128:(i + 1) * 128], wkb[i * 128:(i + 1) * 128])
            elif has_last:
                o = 384 - f0
                wcat[r0:r0 + nr, (48 + p) * 128:(49 + p) * 128] = jnp.concatenate(
                    [fa[:, o:o + 64], fb[:, o:o + 64]], axis=1).astype(BF)

    def colsum(v):
        p = [v[64 * i:64 * (i + 1)] for i in range(7)]
        q = ((p[0] + p[1]) + (p[2] + p[3])) + ((p[4] + p[5]) + p[6])
        r = (q[0:8] + q[8:16]) + (q[16:24] + q[24:32])
        r2 = (q[32:40] + q[40:48]) + (q[48:56] + q[56:64])
        return jnp.sum(r + r2, axis=0, keepdims=True)

    def layernorm(c0):
        xc = xt_v[:, pl.ds(c0, 128)].astype(F32)
        mu = colsum(xc) * (1.0 / D)
        x0 = xc - mu
        var = colsum(x0 * x0) * (1.0 / D)
        xn = x0 * jax.lax.rsqrt(var + 1e-5)
        for t in range(3):
            xn_ref[pl.ds(c0, 128), t * 128:(t + 1) * 128] = xn[t * 128:(t + 1) * 128, :].T
        xl = xn[384:448, :]
        xn_ref[pl.ds(c0, 128), 384:512] = jnp.concatenate([xl, xl], axis=0).T

    att_ref[...] = jnp.zeros((128, DP), BF)
    y_ref[...] = jnp.zeros((D, 128), F32)

    wait(*cv[0], co[0], co[1]); vunits([0], [0, 1])
    wait(*cv[1]); vunits([1], [0, 1])
    wait(co[2], co[3]); vunits([0, 1], [2, 3])
    wait(*cv[2]); vunits([2], [0, 1, 2, 3])
    wait(co[4], co[5]); vunits([0, 1, 2], [4, 5])
    wait(*cv[3], co[6], co[7]); vunits([0, 1, 2], [6, 7])
    vunits([3], [0, 1, 2, 3, 4, 5, 6, 7])

    wait(*cq[0], *cq[3], *ck[0]); split_q(0); kunit(0, 128, 0, 128); split_q(3)
    wait(*cq[1]); split_q(1); kunit(0, 128, 384, 64); kunit(0, 128, 128, 128)
    wait(*ck[1]); kunit(128, 128, 0, 256)
    wait(*cq[2]); split_q(2); kunit(128, 128, 384, 64); kunit(0, 256, 256, 128)
    wait(*ck[2]); kunit(256, 128, 0, 448)
    wait(*ck[3], cx0); layernorm(0); kunit(384, 64, 0, 448)
    wait(c1, c2)

    lane = jax.lax.broadcasted_iota(jnp.int32, (8, 128), 1)
    sub = jax.lax.broadcasted_iota(jnp.int32, (8, 128), 0)
    diag_mask = (lane & 7) <= sub
    lane40 = jax.lax.broadcasted_iota(jnp.int32, (40, 128), 1)
    lo_masks = {}

    def lo_mask(nr):
        if nr not in lo_masks:
            lo_masks[nr] = jax.lax.broadcasted_iota(jnp.int32, (nr, 128), 1) < 64
        return lo_masks[nr]

    def project(hb, rowmap, part, t, ci):
        tile0 = part * NTP + t * NH + ci * 4
        y = jnp.dot(hb, wcat[:, tile0 * 128:(tile0 + 4) * 128], preferred_element_type=F32)
        if t < 3:
            for q in range(2):
                a = ci * 4 + 2 * q
                ya = y[:, (2 * q) * 128:(2 * q + 1) * 128]
                yb = y[:, (2 * q + 1) * 128:(2 * q + 2) * 128]
                for r, (ks, vs, jh) in enumerate(rowmap):
                    blk = jnp.concatenate([ya[8 * r:8 * r + 8], yb[8 * r:8 * r + 8]], axis=0)
                    dst = ks if part == 0 else vs
                    dst[jh * 128 + a * 8:jh * 128 + a * 8 + 16, t * 128:(t + 1) * 128] = blk.astype(BF)
        else:
            lo = lo_mask(hb.shape[0])
            for q in range(4):
                a = 2 * (ci * 4 + q)
                yt = y[:, q * 128:(q + 1) * 128]
                ya = jnp.where(lo, yt, 0.0)
                yb = jnp.where(lo, 0.0, yt)
                for r, (ks, vs, jh) in enumerate(rowmap):
                    blk = jnp.concatenate([ya[8 * r:8 * r + 8], yb[8 * r:8 * r + 8]], axis=0)
                    dst = ks if part == 0 else vs
                    dst[jh * 128 + a * 8:jh * 128 + a * 8 + 16, 384:512] = blk.astype(BF)

    def softmax(s):
        tiles, ms = [], []
        for ih in range(5):
            row = []
            for jh in (range(5) if ih == 0 else range(ih + 1)):
                tt = s[8 * ih:8 * ih + 8, 128 * jh:128 * (jh + 1)]
                if ih > 0 and jh == ih:
                    tt = jnp.where(diag_mask, tt, MASK_VAL)
                row.append(tt)
            tiles.append(row)
            ms.append(functools.reduce(jnp.maximum, row))
        m = _grp8_allreduce(jnp.concatenate(ms, axis=0), jnp.maximum, lane40)
        es, ls = [], []
        for ih in range(5):
            mi = m[8 * ih:8 * ih + 8]
            row = [jnp.exp2((tt - mi) * EXP2_SCALE) for tt in tiles[ih]]
            es.append(row)
            ls.append(functools.reduce(jnp.add, row))
        r = 1.0 / _grp8_allreduce(jnp.concatenate(ls, axis=0), jnp.add, lane40)
        rows = []
        for ih in range(5):
            ri = r[8 * ih:8 * ih + 8]
            row = [e * ri for e in es[ih]]
            row += [jnp.zeros((8, 128), F32)] * (5 - len(row))
            rows.append(jnp.concatenate(row, axis=1))
        rows.append(jnp.zeros((8, 640), F32))
        return jnp.concatenate(rows, axis=0).astype(BF)

    def pv(p, vs, t):
        o = jnp.dot(p, vs[:, t * 128:(t + 1) * 128], preferred_element_type=F32)[0:40]
        if t == 3:
            o = o + pltpu.roll(o, 64, axis=1)
        return o

    def ffn1(g, n0, nn):
        xb = xn_ref[pl.ds(pl.multiple_of(g * 128, 128), 128), :].astype(BF)[:, 0:D]
        h = jnp.dot(xb, w1_v[:, n0 * 128:(n0 + nn) * 128], preferred_element_type=F32)
        h1_ref[:, n0 * 128:(n0 + nn) * 128] = (h * jax.nn.sigmoid(h)).astype(BF)

    def ffn2(r0, rows):
        y_ref[r0:r0 + rows, :] = _nt(w2t_v[r0:r0 + rows, :], h1_ref[...])

    def out_copy(g):
        c0 = pl.multiple_of(g * 128, 128)
        return pltpu.make_async_copy(xt_v.at[:, pl.ds(c0, 128)], o_hbm.at[:, pl.ds(c0, 128)], sems.at[so + g % 2])

    def out_stage(gs, gx):
        c0 = pl.multiple_of(gx * 128, 128)
        c1 = pl.multiple_of(gs * 128, 128)
        for t in range(4):
            n = 128 if t < 3 else 64
            at = att_ref[:, t * 128:(t + 1) * 128].astype(F32).T[0:n]
            res = at + y_ref[t * 128:t * 128 + n, :] + xt_v[t * 128:t * 128 + n, pl.ds(c0, 128)].astype(F32)
            xt_v[t * 128:t * 128 + n, pl.ds(c1, 128)] = res.astype(BF)

    def step(hproj, hq, rowmap, ks, vs, fillers, side, prog):
        fillers = list(fillers)
        sc, outs, prob = {}, {}, None
        for tok in prog:
            kind = tok[0]
            if kind == "K":
                project(hproj, rowmap, 0, int(tok[1]), int(tok[2]))
            elif kind == "V":
                project(hproj, rowmap, 1, int(tok[1]), int(tok[2]))
            elif kind == "S":
                j = int(tok[1])
                sc[j] = _nt(hq, ks[j * 128:(j + 1) * 128, :])
            elif kind == "M":
                prob = softmax(jnp.concatenate([sc[j] for j in range(5)], axis=1))
            elif kind == "P":
                outs[int(tok[1])] = pv(prob, vs, int(tok[1]))
            elif kind == "F":
                fillers.pop(0)()
            elif side is not None:
                side()
        return jnp.concatenate([outs[t] for t in range(4)], axis=1)

    def group(g, mem):
        gn = jnp.minimum(g + 1, NG - 1)
        f1 = [functools.partial(ffn1, g, n0, nn) for (n0, nn) in F1_PIECES]
        f2 = [functools.partial(ffn2, r0, nr) for (r0, nr) in F2_PIECES]
        fills = [f1[:3], f1[3:], f2[:3], f2[3:]]
        sides = [lambda: out_stage(jnp.where(g > 0, g - 1, NG), jnp.maximum(g - 1, 0)), None,
                 lambda: layernorm(pl.multiple_of(gn * 128, 128)), None]
        for u in range(2):
            t0 = pl.multiple_of(g * 128 + 64 * u, 64)
            ha = jnp.concatenate([mem, xn_ref[pl.ds(t0, 40), :]], axis=0).astype(BF)
            oa = step(ha[:, 0:D], ha,
                      [(ka, va, 0), (ka, va, 1), (ka, va, 2), (ka, va, 3), (ka, va, 4), (kb, vb, 1)],
                      ka, va, fills[2 * u], sides[2 * u], PROG_A)
            memb = oa[0:8]
            att_ref[64 * u:64 * u + 32, :] = oa[8:40].astype(BF)
            hb = jnp.concatenate([memb, xn_ref[pl.ds(t0 + 40, 24), :]], axis=0).astype(BF)
            hq = jnp.concatenate([memb, xn_ref[pl.ds(t0 + 32, 32), :], jnp.zeros((8, DP), F32)], axis=0).astype(BF)
            ob = step(hb[:, 0:D], hq, [(kb, vb, 0), (kb, vb, 2), (kb, vb, 3), (kb, vb, 4)],
                      kb, vb, fills[2 * u + 1], sides[2 * u + 1], PROG_B)
            mem = ob[0:8]
            att_ref[64 * u + 32:64 * u + 64, :] = ob[8:40].astype(BF)

        @pl.when(g == 0)
        def _():
            cxr.wait()

        @pl.when(g > 0)
        def _():
            out_copy(g - 1).start()

        @pl.when(g > 1)
        def _():
            out_copy(g - 2).wait()

        return mem

    m0 = mem0_ref[...].astype(F32)
    ml = m0[:, 384:448]
    jax.lax.fori_loop(0, NG, group, jnp.concatenate([m0[:, 0:384], ml, ml], axis=1))

    out_stage(NG - 1, NG - 1)
    out_copy(NG - 1).start()
    out_copy(NG - 2).wait()
    out_copy(NG - 1).wait()


def _forward(A_x, A_mem0, A_Wq, A_Wk, A_Wv, A_Wo, B_w1, B_w2):
    xt = jnp.swapaxes(A_x, 1, 2).reshape(D, SEQ)
    mem0 = A_mem0.reshape(MM, D)
    wq = A_Wq.reshape(D * NH, DH)
    wk = A_Wk.reshape(D * NH, DH)
    wv = A_Wv.reshape(D * NH, DH)
    wo = jnp.swapaxes(A_Wo, 1, 2).reshape(NH * D, DH)
    w2t = jnp.swapaxes(B_w2, 0, 1)
    hbm = pl.BlockSpec(memory_space=pl.ANY)
    half = pltpu.VMEM((D * NH + 64, 128), BF)
    out = pl.pallas_call(
        _kernel,
        out_shape=jax.ShapeDtypeStruct((D, SEQ), BF),
        in_specs=[hbm, pl.BlockSpec(memory_space=pltpu.VMEM), hbm, hbm, hbm, hbm, hbm, hbm],
        out_specs=hbm,
        scratch_shapes=[
            pltpu.VMEM((D, SEQ + 128), BF),
            half, half, half, half, half, half,
            pltpu.VMEM((NH * D, DH), BF),
            pltpu.VMEM((D, FF), BF), pltpu.VMEM((D, FF), BF),
            pltpu.VMEM((NH * D, DH), BF),
            pltpu.VMEM((D, 2 * NTP * 128), BF),
            pltpu.VMEM((SEQ, DP), F32),
            pltpu.VMEM((640, DP), BF), pltpu.VMEM((640, DP), BF),
            pltpu.VMEM((640, DP), BF), pltpu.VMEM((640, DP), BF),
            pltpu.VMEM((128, DP), BF),
            pltpu.VMEM((D, 128), F32),
            pltpu.VMEM((128, FF), BF),
            pltpu.SemaphoreType.DMA((38,)),
        ],
        compiler_params=pltpu.CompilerParams(vmem_limit_bytes=100 * 1024 * 1024),
    )(xt, mem0, wq, wk, wv, wo, B_w1, w2t)
    return jnp.swapaxes(out.reshape(1, D, SEQ), 1, 2)


@functools.partial(jax.jit, static_argnames=("A_seg_len",))
def pallas_parallel_sum__memory_aug_recurrent_mem_tr__dense_activation_silu__prompt_kernel(
    A_x: jax.Array,
    A_mem0: jax.Array,
    A_Wq: jax.Array,
    A_Wk: jax.Array,
    A_Wv: jax.Array,
    A_Wo: jax.Array,
    A_seg_len: int,
    B_x: jax.Array,
    B_w1: jax.Array,
    B_w2: jax.Array,
):
    assert A_seg_len == SEG and A_x.shape == (1, SEQ, D) and A_mem0.shape == (1, MM, D)
    assert A_Wq.shape == (D, NH, DH) and B_w1.shape == (D, FF)
    return _forward(A_x, A_mem0, A_Wq, A_Wk, A_Wv, A_Wo, B_w1, B_w2)
```
